```python
import jax
import jax.numpy as jnp

def _softmax(x, axis=-1):
    return jax.nn.softmax(x, axis=axis)
def _gelu(x):
    return jax.nn.gelu(x, approximate=True)
def _silu(x):
    return jax.nn.silu(x)
def _sigmoid(x):
    return jax.nn.sigmoid(x)
def _layernorm(x, axis=-1, eps=1e-5):
    m = jnp.mean(x, axis=axis, keepdims=True)
    v = jnp.var(x, axis=axis, keepdims=True)
    return (x - m) / jnp.sqrt(v + eps)
def _scatter_add(tgt, idx, src, axis=0):
    return tgt.at[idx].add(src)
def _segment_sum(src, seg, n):
    return jax.ops.segment_sum(src, seg, n)
class _Rng:
    def __init__(self, key):
        self._k = key
    def _next(self):
        self._k, sub = jax.random.split(self._k)
        return sub
    def normal(self, shape):
        return jax.random.normal(self._next(), shape, dtype=jnp.bfloat16)
    def randint(self, lo, hi, shape):
        return jax.random.randint(self._next(), shape, lo, hi, dtype=jnp.int32)
    def uniform(self, shape, lo=0.0, hi=1.0):
        return jax.random.uniform(self._next(), shape, jnp.bfloat16, lo, hi)
    def permutation(self, n):
        return jax.random.permutation(self._next(), n)


kernel_name = 'concat_heads__spectral_gfnet__compressed_kv_cla__prompt'

def setup_inputs():
    _rng = _Rng(jax.random.key(int.from_bytes(__import__("os").urandom(4), "little")))
    _w = (lambda a: (lambda t: t.astype(jnp.bfloat16) if jnp.issubdtype(t.dtype, jnp.floating) else t)(jnp.asarray(a)))
    def _A_setup():
        B, S, D = 1, 2048, 448
        Df = D // 2 + 1
        return {
            "x": _w((lambda *s: _rng.normal(s) * 0.05)(B, S, D)),
            "w_r": _w((lambda *s: _rng.normal(s) * 0.05)(S, Df) * 0.02),
            "w_i": _w((lambda *s: _rng.normal(s) * 0.05)(S, Df) * 0.02),
        }
    _A_in = _A_setup()

    def _B_setup():
        B, H, Sq, Sk, D, M = 1, 16, 2048, 2048, 256, 448
        Dc = 4 * D
        return {
            "x": _w((lambda *s: _rng.normal(s) * 0.05)(B, Sq, M)),
            "c_kv": _w((lambda *s: _rng.normal(s) * 0.05)(B, Sk, Dc)),
            "w_q": _w((lambda *s: _rng.normal(s) * 0.05)(M, H, D) * (M ** -0.5)),
            "w_uk": _w((lambda *s: _rng.normal(s) * 0.05)(Dc, H, D) * (Dc ** -0.5)),
            "w_uv": _w((lambda *s: _rng.normal(s) * 0.05)(Dc, H, D) * (Dc ** -0.5)),
            "w_o": _w((lambda *s: _rng.normal(s) * 0.05)(H, D, M) * ((H * D) ** -0.5)),
        }
    _B_in = _B_setup()

    return {
        "A_x": _A_in["x"],
        "A_w_r": _A_in["w_r"],
        "A_w_i": _A_in["w_i"],
        "B_x": _B_in["x"],
        "B_c_kv": _B_in["c_kv"],
        "B_w_q": _B_in["w_q"],
        "B_w_uk": _B_in["w_uk"],
        "B_w_uv": _B_in["w_uv"],
        "B_w_o": _B_in["w_o"],
    }

def reference(A_x, A_w_r, A_w_i, B_x, B_c_kv, B_w_q, B_w_uk, B_w_uv, B_w_o):
    def _A_ref(x, w_r, w_i):
        B, S, D = x.shape
        X = (lambda x, axes=(-2,-1): jnp.fft.rfft2(x.astype(jnp.float32), axes=axes))(x, axes=(-2, -1))
        W = w_r + 1j * w_i
        X = X * W
        y = (lambda x, s, axes=(-2,-1): jnp.fft.irfft2(x, s=s, axes=axes).astype(jnp.bfloat16))(X, (S, D), axes=(-2, -1))
        return y

    def _B_ref(x, c_kv, w_q, w_uk, w_uv, w_o):
        B, Sq, M = x.shape[0], x.shape[1], x.shape[2]
        Sk = c_kv.shape[1]
        H, D = w_q.shape[1], w_q.shape[2]
        q = jnp.einsum("bqm,mhd->bhqd", x, w_q)
        k = jnp.einsum("bkc,chd->bhkd", c_kv, w_uk)
        v = jnp.einsum("bkc,chd->bhkd", c_kv, w_uv)
        scores = jnp.einsum("bhqd,bhkd->bhqk", q, k) * (D ** -0.5)
        off = Sk - Sq
        qi = jnp.arange(Sq)[:, None]
        kj = jnp.arange(Sk)[None, :]
        cmask = kj <= (qi + off)
        scores = jnp.where(cmask[None, None], scores, -1e9)
        p = _softmax(scores, axis=-1)
        ctx = jnp.einsum("bhqk,bhkd->bhqd", p, v)
        return jnp.einsum("bhqd,hdm->bqm", ctx, w_o)

    a = _A_ref(A_x, A_w_r, A_w_i)
    b = _B_ref(B_x, B_c_kv, B_w_q, B_w_uk, B_w_uv, B_w_o)
    return jnp.concatenate([a, b], axis=-1)
```

```python
import functools
import numpy as np
import jax
import jax.numpy as jnp
from jax import lax
from jax.experimental import pallas as pl
from jax.experimental.pallas import tpu as pltpu

S = 2048
M = 448
H = 16
D = 256
DC = 1024
DF = M // 2 + 1
DFP = 256
R = 16
N2 = S // R
BQ = 256
F32 = jnp.float32
BF16 = jnp.bfloat16
NT = (((1,), (1,)), ((), ()))
TN = (((0,), (0,)), ((), ()))
LOG2E = 1.4426950408889634


def _consts():
    m = np.arange(M, dtype=np.float64)[:, None]
    k = np.arange(DF, dtype=np.float64)[None, :]
    ang = 2.0 * np.pi * ((m * k) % M) / M
    f1 = np.zeros((M, 2 * DFP), np.float64)
    f1[:, :DF] = np.cos(ang)
    f1[:, DFP:DFP + DF] = -np.sin(ang)
    f1[:, DFP] = 0.0
    f1[:, DFP + DF - 1] = 0.0
    ck = np.full((DF, 1), 2.0)
    ck[0] = 1.0
    ck[DF - 1] = 1.0
    fi = np.zeros((2 * DFP, M), np.float64)
    fi[:DF] = ck * np.cos(ang).T / M
    fi[DFP:DFP + DF] = -ck * np.sin(ang).T / M
    fi[DFP] = 0.0
    fi[DFP + DF - 1] = 0.0
    k1 = np.arange(R)[:, None, None]
    k2 = np.arange(N2)[None, :, None]
    n2 = np.arange(N2)[None, None, :]
    a = 2.0 * np.pi * ((n2 * (k1 + R * k2)) % S) / S
    gr, gi = np.cos(a), -np.sin(a)
    g = np.concatenate([np.concatenate([gr, -gi], 2), np.concatenate([gi, gr], 2)], 1)
    hr, hi = np.swapaxes(gr, 1, 2) / S, -np.swapaxes(gi, 1, 2) / S
    gin = np.concatenate([np.concatenate([hr, -hi], 2), np.concatenate([hi, hr], 2)], 1)
    cast = lambda t: t.astype(np.float32).astype(jnp.bfloat16)
    pm = np.zeros((128, 128))
    for k1_ in range(R):
        for j in range(8):
            pm[k1_ * 8 + j, k1_ + R * j] = 1.0
    return cast(f1), cast(fi), cast(g), cast(gin), cast(pm)


_C8 = float(np.sqrt(0.5))
_C16 = float(np.cos(np.pi / 8))
_S16 = float(np.sin(np.pi / 8))


def _cmul_w16(z, e, sgn):
    re, im = z
    e %= 16
    if e == 0:
        return z
    if e == 4:
        return (-sgn * im, sgn * re) if sgn == 1 else (im, -re)
    if e == 8:
        return (-re, -im)
    if e == 12:
        return (sgn * im, -sgn * re) if sgn == 1 else (-im, re)
    c = float(np.cos(2 * np.pi * e / 16))
    s = float(sgn * np.sin(2 * np.pi * e / 16))
    if e % 4 == 2:
        if (c > 0) == (s > 0):
            return ((re - im) * c, (re + im) * c)
        return ((re + im) * c, (im - re) * c)
    return (re * c - im * s, re * s + im * c)


def _dft4(a, b, c, d, sgn):
    s0 = (a[0] + c[0], a[1] + c[1])
    d0 = (a[0] - c[0], a[1] - c[1])
    s1 = (b[0] + d[0], b[1] + d[1])
    d1 = (b[0] - d[0], b[1] - d[1])
    y0 = (s0[0] + s1[0], s0[1] + s1[1])
    y2 = (s0[0] - s1[0], s0[1] - s1[1])
    if sgn > 0:
        y1 = (d0[0] - d1[1], d0[1] + d1[0])
        y3 = (d0[0] + d1[1], d0[1] - d1[0])
    else:
        y1 = (d0[0] + d1[1], d0[1] - d1[0])
        y3 = (d0[0] - d1[1], d0[1] + d1[0])
    return y0, y1, y2, y3


def _dft16(x, sgn):
    t = [None] * 4
    for b in range(4):
        t[b] = _dft4(x[b], x[4 + b], x[8 + b], x[12 + b], sgn)
    out = [None] * 16
    for c in range(4):
        u = [_cmul_w16(t[b][c], b * c, sgn) for b in range(4)]
        y = _dft4(u[0], u[1], u[2], u[3], sgn)
        for d in range(4):
            out[c + 4 * d] = y[d]
    return out


def _unpack(b, hi_shift):
    w = lax.shift_left(lax.shift_right_logical(b, hi_shift), jnp.uint32(16))
    return pltpu.bitcast(w, F32).astype(BF16)


def _kernel(ax_hbm, wr_hbm, wi_hbm, x_hbm, c_hbm, wq_hbm, wuk_hbm, wuv_hbm, wo_hbm,
            f1_hbm, fi_hbm, g_hbm, gn_hbm, pm_hbm, out_ref,
            ax_v, wr_v, wi_v, x_v, c_v, wq_v, wuk_v, wuv_v, wo_v,
            f1_v, fi_v, g_v, gn_v, pm_v, xt_v, wp_v,
            y_v, z_v, t_v, yb_v,
            q_v, k_v, v_v, acc_v,
            sem_a, sem_w, sem_wo):
    wq32 = wq_hbm.bitcast(jnp.uint32)
    wuk32 = wuk_hbm.bitcast(jnp.uint32)
    wuv32 = wuv_hbm.bitcast(jnp.uint32)

    def wcopies(p):
        return (pltpu.make_async_copy(wq32.at[:, p, :], wq_v.at[p], sem_w.at[p, 0]),
                pltpu.make_async_copy(wuk32.at[:, p, :], wuk_v.at[p], sem_w.at[p, 1]),
                pltpu.make_async_copy(wuv32.at[:, p, :], wuv_v.at[p], sem_w.at[p, 2]))

    def wocopy(h):
        return pltpu.make_async_copy(wo_hbm.at[h], wo_v.at[h], sem_wo.at[h])

    a_copies = [
        pltpu.make_async_copy(ax_hbm, ax_v, sem_a.at[0]),
        pltpu.make_async_copy(f1_hbm, f1_v, sem_a.at[1]),
        pltpu.make_async_copy(g_hbm, g_v, sem_a.at[2]),
        pltpu.make_async_copy(gn_hbm, gn_v, sem_a.at[3]),
        pltpu.make_async_copy(fi_hbm, fi_v, sem_a.at[4]),
        pltpu.make_async_copy(x_hbm, xt_v, sem_a.at[5]),
        pltpu.make_async_copy(c_hbm, c_v, sem_a.at[6]),
    ]
    w_copies = [pltpu.make_async_copy(wr_hbm, wr_v, sem_a.at[7]),
                pltpu.make_async_copy(wi_hbm, wi_v, sem_a.at[8]),
                pltpu.make_async_copy(pm_hbm, pm_v, sem_a.at[9])]
    for cp in a_copies[:5]:
        cp.start()
    for cp in w_copies:
        cp.start()
    for cp in a_copies[5:]:
        cp.start()
    for p in range(H // 2):
        for cp in wcopies(p):
            cp.start()
        wocopy(2 * p).start()
        wocopy(2 * p + 1).start()

    a_copies[0].wait()
    a_copies[1].wait()
    y_v[...] = lax.dot_general(ax_v[...], f1_v[...], TN, preferred_element_type=F32)

    def radix(src, dst_store, sgn):
        def body(i, carry):
            r0 = pl.multiple_of(i * 16, 16)
            for j in range(2):
                xs = [src(n1, r0, j) for n1 in range(R)]
                ys = _dft16(xs, sgn)
                for k1 in range(R):
                    dst_store(k1, r0, j, ys[k1])
            return carry
        lax.fori_loop(0, N2 // 16, body, 0)

    def src_f(n1, r0, j):
        rows = pl.ds(n1 * N2 + r0, 16)
        return (y_v[rows, pl.ds(j * 128, 128)], y_v[rows, pl.ds(DFP + j * 128, 128)])

    def dst_f(k1, r0, j, y):
        z_v[k1, pl.ds(r0, 16), pl.ds(j * 128, 128)] = y[0].astype(BF16)
        z_v[k1, pl.ds(N2 + r0, 16), pl.ds(j * 128, 128)] = y[1].astype(BF16)

    radix(src_f, dst_f, -1)

    a_copies[2].wait()
    a_copies[3].wait()
    for cp in w_copies:
        cp.wait()

    def wperm(c, carry):
        for part, wsrc in enumerate((wr_v, wi_v)):
            wt = wsrc[:, pl.ds(pl.multiple_of(c * 128, 128), 128)]
            r = lax.dot_general(pm_v[...], wt, NT, preferred_element_type=F32)
            r = jnp.pad(r, ((0, 0), (0, DFP - DF)))
            for k1 in range(R):
                wp_v[k1, pl.ds(part * N2 + pl.multiple_of(c * 8, 8), 8), :] = r[k1 * 8:(k1 + 1) * 8]
        return carry
    lax.fori_loop(0, 16, wperm, 0)

    def spec(m, carry):
        for half in range(2):
            k1 = 2 * m + half
            wrf = wp_v[k1, 0:N2, :]
            wif = wp_v[k1, N2:2 * N2, :]
            x2 = jnp.dot(g_v[k1], z_v[k1], preferred_element_type=F32)
            xr, xi = x2[:N2], x2[N2:]
            ur = (xr * wrf - xi * wif).astype(BF16)
            ui = (xr * wif + xi * wrf).astype(BF16)
            u = jnp.concatenate([ur, ui], axis=0)
            t_v[k1] = jnp.dot(gn_v[k1], u, preferred_element_type=F32)
        return carry
    lax.fori_loop(0, 8, spec, 0)

    def src_i(k1, r0, j):
        return (t_v[k1, pl.ds(r0, 16), pl.ds(j * 128, 128)],
                t_v[k1, pl.ds(N2 + r0, 16), pl.ds(j * 128, 128)])

    def dst_i(n1, r0, j, y):
        rows = pl.ds(n1 * N2 + r0, 16)
        yb_v[rows, pl.ds(j * 128, 128)] = y[0].astype(BF16)
        yb_v[rows, pl.ds(DFP + j * 128, 128)] = y[1].astype(BF16)

    radix(src_i, dst_i, 1)
    a_copies[4].wait()
    out_ref[:, 0:M] = jnp.dot(yb_v[...], fi_v[...], preferred_element_type=F32).astype(BF16)

    a_copies[5].wait()
    x_v[...] = xt_v[...].T
    a_copies[6].wait()
    acc_v[...] = jnp.zeros_like(acc_v)
    qscale = float(D ** -0.5) * LOG2E

    def head(h, carry):
        p = h // 2
        odd = h % 2

        @pl.when(odd == 0)
        def _():
            for cp in wcopies(p):
                cp.wait()
        wocopy(h).wait()
        sh = (odd * 16).astype(jnp.uint32)
        wq = _unpack(wq_v[p], sh)
        q_v[...] = (jnp.dot(x_v[...], wq, preferred_element_type=F32) * qscale).astype(BF16)
        k_v[...] = jnp.dot(c_v[...], _unpack(wuk_v[p], sh), preferred_element_type=F32).astype(BF16)
        v_v[...] = jnp.dot(c_v[...], _unpack(wuv_v[p], sh), preferred_element_type=F32).astype(BF16)
        wo = wo_v[h]
        for i in range(S // BQ):
            q = q_v[pl.ds(i * BQ, BQ), :]
            row = lax.broadcasted_iota(jnp.int32, (BQ, BQ), 0)
            col = lax.broadcasted_iota(jnp.int32, (BQ, BQ), 1)
            sd = lax.dot_general(q, k_v[pl.ds(i * BQ, BQ), :], NT, preferred_element_type=F32)
            sd = jnp.where(col <= row, sd, -1e9)
            m = jnp.max(sd, axis=1, keepdims=True)
            if i > 0:
                so = lax.dot_general(q, k_v[pl.ds(0, i * BQ), :], NT, preferred_element_type=F32)
                m = jnp.maximum(m, jnp.max(so, axis=1, keepdims=True))
            pd = jnp.exp2(sd - m)
            l = jnp.sum(pd, axis=1, keepdims=True)
            o = jnp.dot(pd.astype(BF16), v_v[pl.ds(i * BQ, BQ), :], preferred_element_type=F32)
            if i > 0:
                po = jnp.exp2(so - m)
                l = l + jnp.sum(po, axis=1, keepdims=True)
                o = o + jnp.dot(po.astype(BF16), v_v[pl.ds(0, i * BQ), :], preferred_element_type=F32)
            ctx = (o / l).astype(BF16)
            acc_v[pl.ds(i * BQ, BQ), :] += lax.dot_general(ctx, wo, NT, preferred_element_type=F32)
        return carry
    lax.fori_loop(0, H, head, 0)
    out_ref[:, M:2 * M] = acc_v[...].astype(BF16)


@jax.jit
def pallas_concat_heads__spectral_gfnet__compressed_kv_cla__prompt_kernel(
        A_x, A_w_r, A_w_i, B_x, B_c_kv, B_w_q, B_w_uk, B_w_uv, B_w_o):
    f1, fi, g, gin, pm = _consts()
    u32 = jnp.uint32
    any_spec = pl.BlockSpec(memory_space=pltpu.HBM)
    scratch = [
        pltpu.VMEM((M, S), BF16),
        pltpu.VMEM((DF, S), BF16),
        pltpu.VMEM((DF, S), BF16),
        pltpu.VMEM((S, M), BF16),
        pltpu.VMEM((S, DC), BF16),
        pltpu.VMEM((H // 2, M, D), u32),
        pltpu.VMEM((H // 2, DC, D), u32),
        pltpu.VMEM((H // 2, DC, D), u32),
        pltpu.VMEM((H, M, D), BF16),
        pltpu.VMEM((M, 2 * DFP), BF16),
        pltpu.VMEM((2 * DFP, M), BF16),
        pltpu.VMEM((R, 2 * N2, 2 * N2), BF16),
        pltpu.VMEM((R, 2 * N2, 2 * N2), BF16),
        pltpu.VMEM((128, 128), BF16),
        pltpu.VMEM((M, S), BF16),
        pltpu.VMEM((R, 2 * N2, DFP), F32),
        pltpu.VMEM((S, 2 * DFP), F32),
        pltpu.VMEM((R, 2 * N2, DFP), BF16),
        pltpu.VMEM((R, 2 * N2, DFP), F32),
        pltpu.VMEM((S, 2 * DFP), BF16),
        pltpu.VMEM((S, D), BF16),
        pltpu.VMEM((S, D), BF16),
        pltpu.VMEM((S, D), BF16),
        pltpu.VMEM((S, M), F32),
        pltpu.SemaphoreType.DMA((10,)),
        pltpu.SemaphoreType.DMA((H // 2, 3)),
        pltpu.SemaphoreType.DMA((H,)),
    ]
    out = pl.pallas_call(
        _kernel,
        out_shape=jax.ShapeDtypeStruct((S, 2 * M), BF16),
        in_specs=[any_spec] * 14,
        out_specs=pl.BlockSpec(memory_space=pltpu.VMEM),
        scratch_shapes=scratch,
        compiler_params=pltpu.CompilerParams(vmem_limit_bytes=120 * 2**20),
        name="fused",
    )(A_x.reshape(S, M).T, A_w_r.T, A_w_i.T,
      B_x.reshape(S, M).T, B_c_kv.reshape(S, DC), B_w_q, B_w_uk, B_w_uv, jnp.swapaxes(B_w_o, 1, 2),
      jnp.asarray(f1), jnp.asarray(fi), jnp.asarray(g), jnp.asarray(gin), jnp.asarray(pm))
    return out.reshape(1, S, 2 * M)
```

```python
import functools
import numpy as np
import jax
import jax.numpy as jnp
from jax import lax
from jax.experimental import pallas as pl
from jax.experimental.pallas import tpu as pltpu

S = 2048
M = 448
H = 16
D = 256
DC = 1024
DF = M // 2 + 1
DFP = 256
R = 16
N2 = S // R
BQ = 256
F32 = jnp.float32
BF16 = jnp.bfloat16
NT = (((1,), (1,)), ((), ()))
TN = (((0,), (0,)), ((), ()))
LOG2E = 1.4426950408889634


def _consts():
    m = np.arange(M, dtype=np.float64)[:, None]
    k = np.arange(DF, dtype=np.float64)[None, :]
    ang = 2.0 * np.pi * ((m * k) % M) / M
    f1 = np.zeros((M, 2 * DFP), np.float64)
    f1[:, :DF] = np.cos(ang)
    f1[:, DFP:DFP + DF] = -np.sin(ang)
    f1[:, DFP] = 0.0
    f1[:, DFP + DF - 1] = 0.0
    ck = np.full((DF, 1), 2.0)
    ck[0] = 1.0
    ck[DF - 1] = 1.0
    fi = np.zeros((2 * DFP, M), np.float64)
    fi[:DF] = ck * np.cos(ang).T / M
    fi[DFP:DFP + DF] = -ck * np.sin(ang).T / M
    fi[DFP] = 0.0
    fi[DFP + DF - 1] = 0.0
    k1 = np.arange(R)[:, None, None]
    k2 = np.arange(N2)[None, :, None]
    n2 = np.arange(N2)[None, None, :]
    a = 2.0 * np.pi * ((n2 * (k1 + R * k2)) % S) / S
    gr, gi = np.cos(a), -np.sin(a)
    g = np.concatenate([np.concatenate([gr, -gi], 2), np.concatenate([gi, gr], 2)], 1)
    perm = np.arange(2 * N2).reshape(2, N2 // 8, 8).transpose(1, 0, 2).reshape(-1)
    g = g[:, :, perm]
    hr, hi = np.swapaxes(gr, 1, 2) / S, -np.swapaxes(gi, 1, 2) / S
    gin = np.concatenate([np.concatenate([hr, -hi], 2), np.concatenate([hi, hr], 2)], 1)
    def cast(t):
        b = np.ascontiguousarray(t.astype(np.float32).astype(jnp.bfloat16)).view(np.uint16).astype(np.uint32)
        return b[..., 0::2, :] | (b[..., 1::2, :] << 16)
    pm = np.zeros((128, 128))
    for k1_ in range(R):
        for j in range(8):
            pm[k1_ * 8 + j, k1_ + R * j] = 1.0
    return cast(f1), cast(np.ascontiguousarray(fi.T)), cast(g), cast(gin), cast(pm)


_C8 = float(np.sqrt(0.5))
_C16 = float(np.cos(np.pi / 8))
_S16 = float(np.sin(np.pi / 8))


def _cmul_w16(z, e, sgn):
    re, im = z
    e %= 16
    if e == 0:
        return z
    if e == 4:
        return (-sgn * im, sgn * re) if sgn == 1 else (im, -re)
    if e == 8:
        return (-re, -im)
    if e == 12:
        return (sgn * im, -sgn * re) if sgn == 1 else (-im, re)
    c = float(np.cos(2 * np.pi * e / 16))
    s = float(sgn * np.sin(2 * np.pi * e / 16))
    if e % 4 == 2:
        if (c > 0) == (s > 0):
            return ((re - im) * c, (re + im) * c)
        return ((re + im) * c, (im - re) * c)
    return (re * c - im * s, re * s + im * c)


def _dft4(a, b, c, d, sgn):
    s0 = (a[0] + c[0], a[1] + c[1])
    d0 = (a[0] - c[0], a[1] - c[1])
    s1 = (b[0] + d[0], b[1] + d[1])
    d1 = (b[0] - d[0], b[1] - d[1])
    y0 = (s0[0] + s1[0], s0[1] + s1[1])
    y2 = (s0[0] - s1[0], s0[1] - s1[1])
    if sgn > 0:
        y1 = (d0[0] - d1[1], d0[1] + d1[0])
        y3 = (d0[0] + d1[1], d0[1] - d1[0])
    else:
        y1 = (d0[0] + d1[1], d0[1] - d1[0])
        y3 = (d0[0] - d1[1], d0[1] + d1[0])
    return y0, y1, y2, y3


def _dft16(x, sgn):
    t = [None] * 4
    for b in range(4):
        t[b] = _dft4(x[b], x[4 + b], x[8 + b], x[12 + b], sgn)
    out = [None] * 16
    for c in range(4):
        u = [_cmul_w16(t[b][c], b * c, sgn) for b in range(4)]
        y = _dft4(u[0], u[1], u[2], u[3], sgn)
        for d in range(4):
            out[c + 4 * d] = y[d]
    return out


NEG = -1e9 * LOG2E
QSCALE = float(D ** -0.5) * LOG2E
HB = BQ // 2
KH = DC // 2
MH = M // 2
NB = S // BQ
U32 = jnp.uint32
OPLACE = {7: (0, 1, 2, 3, 4, 5)}
CARRY = (6, 7)
GR = 16
UCH = 16
UPOS = "a"
ST_Q = 1
ST_O = 0


def _ds(start, size, mult=None):
    if not isinstance(start, int):
        start = pl.multiple_of(start, mult or size)
    return pl.ds(start, size)


def _ld(ref, pre, r0, nr, cols=slice(None)):
    return pltpu.bitcast(ref[pre + (_ds(r0 // 2, nr // 2, 8), cols)], BF16)


def _st(ref, pre, r0, val, cols=slice(None)):
    ref[pre + (_ds(r0 // 2, val.shape[0] // 2, 8), cols)] = pltpu.bitcast(val.astype(BF16), U32)


def _kernel(ax_hbm, wr_hbm, wi_hbm, x_hbm, c_hbm, wq_hbm, wuk_hbm, wuv_hbm, wo_hbm,
            f1_hbm, fi_hbm, g_hbm, gn_hbm, pm_hbm, out_hbm,
            ax_v, wr_v, wi_v, x_v, c_v, wq_v, wuk_v, wuv_v, wo_v,
            f1_v, fi_v, g_v, gn_v, pm_v, xt_v, wp_v,
            y_v, z_v, t_v, yf_v,
            q_v, k_v, v_v, ctx_v, wqb_v, bc_v, ac_v, xc_v, pa_v, pb_v,
            acc_v, woc_v, ot_v, out_v,
            sem_a, sem_w, sem_wo, sem_o):
    wq32 = wq_hbm.bitcast(U32)
    wuk32 = wuk_hbm.bitcast(U32)
    wuv32 = wuv_hbm.bitcast(U32)
    wo32 = wo_hbm.bitcast(U32)

    def wcopies(p):
        return (pltpu.make_async_copy(wq32.at[:, p, :], wq_v.at[p], sem_w.at[p, 0]),
                pltpu.make_async_copy(wuk32.at[:, p, :], wuk_v.at[p], sem_w.at[p, 1]),
                pltpu.make_async_copy(wuv32.at[:, p, :], wuv_v.at[p], sem_w.at[p, 2]))

    def wocopy(h):
        return pltpu.make_async_copy(wo32.at[h], wo_v.at[h], sem_wo.at[h])

    def ocopy(i):
        rows = _ds(i * BQ, BQ)
        return pltpu.make_async_copy(out_v.at[rows], out_hbm.at[rows], sem_o.at[i])

    cp_ax = pltpu.make_async_copy(ax_hbm.bitcast(U32), ax_v, sem_a.at[0])
    cp_f1 = pltpu.make_async_copy(f1_hbm, f1_v, sem_a.at[1])
    cp_g = pltpu.make_async_copy(g_hbm, g_v, sem_a.at[2])
    cp_gn = pltpu.make_async_copy(gn_hbm, gn_v, sem_a.at[3])
    cp_fi = pltpu.make_async_copy(fi_hbm, fi_v, sem_a.at[4])
    cp_x = pltpu.make_async_copy(x_hbm.bitcast(U32), xt_v, sem_a.at[5])
    cp_c = pltpu.make_async_copy(c_hbm.bitcast(U32), c_v, sem_a.at[6])
    cp_wr = pltpu.make_async_copy(wr_hbm, wr_v, sem_a.at[7])
    cp_wi = pltpu.make_async_copy(wi_hbm, wi_v, sem_a.at[8])
    cp_pm = pltpu.make_async_copy(pm_hbm, pm_v, sem_a.at[9])

    def _halves(w):
        return (pltpu.bitcast(w << 16, F32), pltpu.bitcast(w & U32(0xFFFF0000), F32))

    def combos(src, dst, i, width):
        ch = 16
        for r in range(0, HB // 2, ch):
            top = _ds(i * (BQ // 2) + r, ch, 8)
            bot = _ds(i * (BQ // 2) + HB // 2 + r, ch, 8)
            a11 = _halves(src[top, pl.ds(0, width)])
            a12 = _halves(src[top, pl.ds(width, width)])
            a21 = _halves(src[bot, pl.ds(0, width)])
            a22 = _halves(src[bot, pl.ds(width, width)])
            terms = ((a11, a22, 1), (a21, a22, 1), (a11, a12, 1), (a21, a11, -1), (a12, a22, -1))
            for j, (u, v, sg) in enumerate(terms):
                t = [u[e] + v[e] if sg > 0 else u[e] - v[e] for e in range(2)]
                dst[j, _ds(i * (HB // 2) + r, ch, 8), :] = pltpu.bitcast(
                    pltpu.pack_elementwise(t, packed_dtype=BF16), U32)

    def latent_combos(i):
        combos(c_v, ac_v, i, KH)

    def unpack_weights(p, odd):
        sh = (odd * 16).astype(U32) if not isinstance(odd, int) else U32(odd * 16)
        unf = lambda t: pltpu.bitcast(lax.shift_left(lax.shift_right_logical(t, sh), U32(16)), F32)
        if ST_Q:
            for r in range(0, D, UCH):
                b1 = unf(wq_v[p, pl.ds(r, UCH), :])
                b11, b12 = b1[:, :128], b1[:, 128:]
                if D + r < M:
                    b2 = unf(wq_v[p, pl.ds(D + r, UCH), :])
                    b21, b22 = b2[:, :128], b2[:, 128:]
                    cmb = (b11 + b22, b11, b12 - b22, b21 - b11, b22, b11 + b12, b21 + b22)
                else:
                    zero = jnp.zeros_like(b11)
                    cmb = (b11, b11, b12, -b11, zero, b11 + b12, zero)
                for j, t in enumerate(cmb):
                    _st(wqb_v, (j,), r, t)
        else:
            _st(wqb_v, (), 0, unf(wq_v[p]))
        for r in range(0, KH, UCH):
            b11 = unf(wuk_v[p, pl.ds(r, UCH), :])
            b21 = unf(wuk_v[p, pl.ds(KH + r, UCH), :])
            b12 = unf(wuv_v[p, pl.ds(r, UCH), :])
            b22 = unf(wuv_v[p, pl.ds(KH + r, UCH), :])
            for j, t in enumerate((b11 + b22, b11, b12 - b22, b21 - b11, b22, b11 + b12, b21 + b22)):
                _st(bc_v, (j,), r, t)

    def x_combos(i):
        combos(x_v, xc_v, i, D)

    def proj_q(i):
        if not ST_Q:
            r = jnp.dot(_ld(x_v, (), i * BQ, BQ, pl.ds(0, M)), _ld(wqb_v, (), 0, M), preferred_element_type=F32)
            _st(q_v, (), i * BQ, r * QSCALE)
            return
        top, bot, ar = i * BQ, i * BQ + HB, i * HB
        mm = lambda a, j: jnp.dot(a, _ld(wqb_v, (j,), 0, D), preferred_element_type=F32)
        xc = lambda j: _ld(xc_v, (j,), ar, HB)
        m7 = mm(xc(4), 6)
        m1 = mm(xc(0), 0)
        m4 = mm(_ld(x_v, (), bot, HB, pl.ds(D, D)), 3)
        m5 = mm(xc(2), 4)
        m3 = mm(_ld(x_v, (), top, HB, pl.ds(0, D)), 2)
        _st(q_v, (), top, jnp.concatenate([m1 + m4 - m5 + m7, m3 + m5], axis=1) * QSCALE)
        m2 = mm(xc(1), 1)
        m6 = mm(xc(3), 5)
        _st(q_v, (), bot, jnp.concatenate([m2 + m4, m1 - m2 + m3 + m6], axis=1) * QSCALE)

    def proj_kv(i):
        top, bot, ar = i * BQ, i * BQ + HB, i * HB
        mm = lambda a, j: jnp.dot(a, _ld(bc_v, (j,), 0, KH), preferred_element_type=F32)
        ac = lambda j: _ld(ac_v, (j,), ar, HB)
        m7 = mm(ac(4), 6)
        m1 = mm(ac(0), 0)
        m4 = mm(_ld(c_v, (), bot, HB, pl.ds(KH, KH)), 3)
        m5 = mm(ac(2), 4)
        _st(k_v, (), top, m1 + m4 - m5 + m7)
        m3 = mm(_ld(c_v, (), top, HB, pl.ds(0, KH)), 2)
        _st(v_v, (), top, m3 + m5)
        m2 = mm(ac(1), 1)
        _st(k_v, (), bot, m2 + m4)
        m6 = mm(ac(3), 5)
        _st(v_v, (), bot, m1 - m2 + m3 + m6)

    cp_ax.start()
    cp_f1.start()
    cp_ax.wait()
    cp_f1.wait()
    for cp in (cp_pm, cp_wr, cp_wi):
        cp.start()

    def a1(i, carry):
        n = _ds(i * 512, 512)
        for step, cps in ((1, (cp_g,)), (2, (cp_gn,)), (3, (cp_x,))):
            @pl.when(i == step)
            def _():
                for cp in cps:
                    cp.start()
        acc_v[:, n] = jnp.zeros((M, 512), F32)
        ctx_v[_ds(i * 256, 256), :] = jnp.zeros((256, D), U32)
        y_v[n, :] = lax.dot_general(_ld(ax_v, (), 0, M, n), _ld(f1_v, (), 0, M), TN, preferred_element_type=F32)
        return carry
    lax.fori_loop(0, 4, a1, 0)

    def radix(src, dst_store, sgn, filler):
        def body(i, carry):
            r0 = pl.multiple_of(i * 8, 8)
            for j in range(2):
                xs = [src(n1, r0, j) for n1 in range(R)]
                ys = _dft16(xs, sgn)
                for k1 in range(R):
                    dst_store(k1, r0, j, ys[k1])
            filler(i)
            return carry
        lax.fori_loop(0, N2 // 8, body, 0)

    def src_f(n1, r0, j):
        rows = _ds(n1 * N2 + r0, 8)
        return (y_v[rows, pl.ds(j * 128, 128)], y_v[rows, pl.ds(DFP + j * 128, 128)])

    def dst_f(k1, r0, j, y):
        _st(z_v, (k1,), 2 * r0, jnp.concatenate(y, axis=0), pl.ds(j * 128, 128))

    def wperm(c):
        for part, wsrc in enumerate((wr_v, wi_v)):
            wt = wsrc[:, _ds(c * 128, 128)]
            r = lax.dot_general(_ld(pm_v, (), 0, 128), wt, NT, preferred_element_type=F32)
            r = jnp.pad(r, ((0, 0), (0, DFP - DF)))
            for k1 in range(R):
                wp_v[k1, _ds(part * N2 + c * 8, 8), :] = r[k1 * 8:(k1 + 1) * 8]

    for cp in (cp_pm, cp_wr, cp_wi):
        cp.wait()
    w0 = wcopies(0)
    cp_c.start()

    radix(src_f, dst_f, -1, wperm)

    def fwd(k1):
        return jnp.dot(_ld(g_v, (k1,), 0, 2 * N2), _ld(z_v, (k1,), 0, 2 * N2), preferred_element_type=F32)

    cp_g.wait()
    cp_gn.wait()
    cp_x.wait()
    for cp in (cp_fi, w0[0], w0[1], w0[2], wocopy(0), wocopy(1)):
        cp.start()

    def spec(m, carry):
        n = _ds(m * 256, 256)
        xt = jnp.concatenate([_ld(xt_v, (), 0, M, n), jnp.zeros((4 * 128 - M, 256), BF16)], axis=0)
        _st(x_v, (), m * 256, xt.T)
        xa = fwd(2 * m)
        xb = fwd(2 * m + 1)
        for k1, x2 in ((2 * m, xa), (2 * m + 1, xb)):
            wrf = wp_v[k1, 0:N2, :]
            wif = wp_v[k1, N2:2 * N2, :]
            xr, xi = x2[:N2], x2[N2:]
            ur = (xr * wrf - xi * wif).astype(BF16)
            ui = (xr * wif + xi * wrf).astype(BF16)
            u = jnp.concatenate([ur, ui], axis=0)
            t_v[k1] = jnp.dot(_ld(gn_v, (k1,), 0, 2 * N2), u, preferred_element_type=F32)
        return carry
    lax.fori_loop(0, R // 2, spec, 0)

    def src_i(k1, r0, j):
        return (t_v[k1, pl.ds(r0, 8), pl.ds(j * 128, 128)],
                t_v[k1, _ds(N2 + r0, 8), pl.ds(j * 128, 128)])

    def dst_i(n1, r0, j, y):
        rows = _ds(n1 * N2 + r0, 8)
        yf_v[rows, pl.ds(j * 128, 128)] = y[0]
        yf_v[rows, pl.ds(DFP + j * 128, 128)] = y[1]

    radix(src_i, dst_i, 1, lambda i: None)
    cp_fi.wait()
    cp_c.wait()
    for cp in w0:
        cp.wait()

    def a5(i, carry):
        n = _ds(i * 512, 512)
        _st(ot_v, (), 0, lax.dot_general(_ld(fi_v, (), 0, M), yf_v[n, :].astype(BF16), NT,
                                         preferred_element_type=F32), n)
        latent_combos(2 * i)
        latent_combos(2 * i + 1)
        x_combos(2 * i)
        x_combos(2 * i + 1)
        return carry
    lax.fori_loop(0, 4, a5, 0)

    row = lax.broadcasted_iota(jnp.int32, (HB, HB), 0)
    col = lax.broadcasted_iota(jnp.int32, (HB, HB), 1)
    tri = col <= row
    p_bufs = (pa_v, pb_v)

    def wo_combos(h):
        if not ST_O:
            return
        for r in range(0, MH, 32):
            a1 = _ld(wo_v, (h,), r, 32).astype(F32)
            a2 = _ld(wo_v, (h,), MH + r, 32).astype(F32)
            a11, a12, a21, a22 = a1[:, :128], a1[:, 128:], a2[:, :128], a2[:, 128:]
            for j, t in enumerate((a11 + a22, a21 + a22, a11, a22, a11 + a12, a21 - a11, a12 - a22)):
                _st(woc_v, (j,), r, t)

    def oproj(i, h):
        if ST_O:
            cols = pl.ds(i * HB, HB)
            for j in range(7):
                acc_v[j, :, cols] += lax.dot_general(_ld(woc_v, (j,), 0, MH), _ld(ctx_v, (j,), i * HB, HB), NT,
                                                     preferred_element_type=F32)
            return
        cols = pl.ds(i * BQ, BQ)
        acc_v[:, cols] += lax.dot_general(h, _ld(ctx_v, (), i * BQ, BQ), NT, preferred_element_type=F32)


    def head(h, carry):
        p = h // 2
        odd = h % 2

        @pl.when(jnp.logical_and(odd == 0, p + 1 < H // 2))
        def _():
            for cp in wcopies(p + 1):
                cp.start()
            wocopy(h + 2).start()
            wocopy(h + 3).start()

        @pl.when(jnp.logical_and(odd == 0, h > 0))
        def _():
            for cp in wcopies(p):
                cp.wait()

        wocopy(h).wait()
        wo_prev = _ld(wo_v, (jnp.maximum(h - 1, 0),), 0, M)
        wo = _ld(wo_v, (h,), 0, M)
        unpack_weights(p, odd)
        for j in CARRY:
            oproj(j, wo_prev)
        proj_q(0)
        proj_kv(0)
        for i in range(NB):
            r0 = i * BQ
            l1 = r0 + HB
            q = _ld(q_v, (), r0, BQ)
            s1 = lax.dot_general(q, _ld(k_v, (), 0, l1), NT, preferred_element_type=F32)
            s2 = lax.dot_general(q[HB:], _ld(k_v, (), l1, HB), NT, preferred_element_type=F32)
            if i + 1 < NB:
                proj_q(i + 1)
                proj_kv(i + 1)
            for j in OPLACE.get(i, ()):
                oproj(j, wo)
            sdl = jnp.where(tri, s1[:HB, r0:], NEG)
            s_lo = jnp.concatenate([s1[:HB, :r0], sdl], axis=1) if i > 0 else sdl
            s_hi = jnp.concatenate([s1[HB:], jnp.where(tri, s2, NEG)], axis=1)
            pb = p_bufs[i % 2]
            ls = []
            for half, s_h in enumerate((s_lo, s_hi)):
                w = s_h.shape[1]
                for g in range(HB // GR):
                    sg = s_h[g * GR:(g + 1) * GR]
                    pg = jnp.exp2(sg - jnp.max(sg, axis=1, keepdims=True))
                    _st(pb, (), half * HB + g * GR, pg, pl.ds(0, w))
                    ls.append(jnp.sum(pg, axis=1, keepdims=True))
            l = jnp.concatenate(ls, axis=0)
            o = jnp.dot(_ld(pb, (), 0, BQ, pl.ds(0, l1)), _ld(v_v, (), 0, l1), preferred_element_type=F32)
            o2 = jnp.dot(_ld(pb, (), HB, HB, pl.ds(l1, HB)), _ld(v_v, (), l1, HB), preferred_element_type=F32)
            o = jnp.concatenate([o[:HB], o[HB:] + o2], axis=0)
            ctx = o / l
            if ST_O:
                b11, b21, b12, b22 = ctx[:HB, :128], ctx[:HB, 128:], ctx[HB:, :128], ctx[HB:, 128:]
                for j, t in enumerate((b11 + b22, b11, b12 - b22, b21 - b11, b22, b11 + b12, b21 + b22)):
                    _st(ctx_v, (j,), i * HB, t)
            else:
                _st(ctx_v, (), r0, ctx)
        return carry

    lax.fori_loop(0, H, head, 0)

    for j in CARRY:
        oproj(j, _ld(wo_v, (H - 1,), 0, M))

    def fin(i, carry):
        cols = _ds(i * BQ, BQ)
        if ST_O:
            hc = _ds(i * HB, HB)
            m1, m2, m3, m4, m5, m6, m7 = (acc_v[j, :, hc] for j in range(7))
            _st(ot_v, (), M, jnp.concatenate([m1 + m4 - m5 + m7, m3 + m5], axis=1), cols)
            _st(ot_v, (), M + MH, jnp.concatenate([m2 + m4, m1 - m2 + m3 + m6], axis=1), cols)
        else:
            _st(ot_v, (), M, acc_v[:, cols], cols)
        out_v[cols, :] = _ld(ot_v, (), 0, 2 * M, cols).T
        ocopy(i).start()
        return carry
    lax.fori_loop(0, NB, fin, 0)
    for i in range(NB):
        ocopy(i).wait()


@jax.jit
def pallas_concat_heads__spectral_gfnet__compressed_kv_cla__prompt_kernel(
        A_x, A_w_r, A_w_i, B_x, B_c_kv, B_w_q, B_w_uk, B_w_uv, B_w_o):
    f1, fi, g, gin, pm = _consts()
    packed = lambda *shape: pltpu.VMEM(shape[:-2] + (shape[-2] // 2, shape[-1]), U32)
    hbm = pl.BlockSpec(memory_space=pltpu.HBM)
    scratch = [
        packed(M, S),
        pltpu.VMEM((DF, S), BF16),
        pltpu.VMEM((DF, S), BF16),
        packed(S, 4 * 128),
        packed(S, DC),
        pltpu.VMEM((H // 2, M, D), U32),
        pltpu.VMEM((H // 2, DC, D), U32),
        pltpu.VMEM((H // 2, DC, D), U32),
        packed(H, M, D),
        packed(M, 2 * DFP),
        packed(M, 2 * DFP),
        packed(R, 2 * N2, 2 * N2),
        packed(R, 2 * N2, 2 * N2),
        packed(128, 128),
        packed(M, S),
        pltpu.VMEM((R, 2 * N2, DFP), F32),
        pltpu.VMEM((S, 2 * DFP), F32),
        packed(R, 2 * N2, DFP),
        pltpu.VMEM((R, 2 * N2, DFP), F32),
        pltpu.VMEM((S, 2 * DFP), F32),
        packed(S, D),
        packed(S, D),
        packed(S, D),
        packed(7, S // 2, D // 2) if ST_O else packed(S, D),
        packed(7, D, D // 2) if ST_Q else packed(M, D),
        packed(7, KH, D),
        packed(5, S // 2, KH),
        packed(5, S // 2, D),
        packed(BQ, S),
        packed(BQ, S),
        pltpu.VMEM((7, MH, S // 2), F32) if ST_O else pltpu.VMEM((M, S), F32),
        packed(7, MH, D // 2),
        packed(2 * M, S),
        pltpu.VMEM((S, 2 * M), BF16),
        pltpu.SemaphoreType.DMA((10,)),
        pltpu.SemaphoreType.DMA((H // 2, 3)),
        pltpu.SemaphoreType.DMA((H,)),
        pltpu.SemaphoreType.DMA((NB,)),
    ]
    out = pl.pallas_call(
        _kernel,
        out_shape=jax.ShapeDtypeStruct((S, 2 * M), BF16),
        in_specs=[hbm] * 14,
        out_specs=hbm,
        scratch_shapes=scratch,
        compiler_params=pltpu.CompilerParams(vmem_limit_bytes=120 * 2**20),
        name="fused",
    )(A_x.reshape(S, M).T, A_w_r.T, A_w_i.T,
      B_x.reshape(S, M).T, B_c_kv.reshape(S, DC), B_w_q, B_w_uk, B_w_uv, jnp.swapaxes(B_w_o, 1, 2),
      jnp.asarray(f1), jnp.asarray(fi), jnp.asarray(g), jnp.asarray(gin), jnp.asarray(pm))
    return out.reshape(1, S, 2 * M)
```

```python
import numpy as np
import jax
import jax.numpy as jnp
from jax import lax
from jax.experimental import pallas as pl
from jax.experimental.pallas import tpu as pltpu

S = 2048
M = 448
H = 16
D = 256
DC = 1024
DF = M // 2 + 1
DFP = 256
R = 16
N2 = S // R
BQ = 256
F32 = jnp.float32
BF16 = jnp.bfloat16
NT = (((1,), (1,)), ((), ()))
TN = (((0,), (0,)), ((), ()))
LOG2E = 1.4426950408889634


def _consts():
    m = np.arange(M, dtype=np.float64)[:, None]
    k = np.arange(DF, dtype=np.float64)[None, :]
    ang = 2.0 * np.pi * ((m * k) % M) / M
    f1 = np.zeros((M, 2 * DFP), np.float64)
    f1[:, :DF] = np.cos(ang)
    f1[:, DFP:DFP + DF] = -np.sin(ang)
    f1[:, DFP] = 0.0
    f1[:, DFP + DF - 1] = 0.0
    ck = np.full((DF, 1), 2.0)
    ck[0] = 1.0
    ck[DF - 1] = 1.0
    fi = np.zeros((2 * DFP, M), np.float64)
    fi[:DF] = ck * np.cos(ang).T / M
    fi[DFP:DFP + DF] = -ck * np.sin(ang).T / M
    fi[DFP] = 0.0
    fi[DFP + DF - 1] = 0.0
    k1 = np.arange(R)[:, None, None]
    k2 = np.arange(N2)[None, :, None]
    n2 = np.arange(N2)[None, None, :]
    a = 2.0 * np.pi * ((n2 * (k1 + R * k2)) % S) / S
    gr, gi = np.cos(a), -np.sin(a)
    g = np.concatenate([np.concatenate([gr, -gi], 2), np.concatenate([gi, gr], 2)], 1)
    perm = np.arange(2 * N2).reshape(2, N2 // 8, 8).transpose(1, 0, 2).reshape(-1)
    g = g[:, :, perm]
    hr, hi = np.swapaxes(gr, 1, 2) / S, -np.swapaxes(gi, 1, 2) / S
    gin = np.concatenate([np.concatenate([hr, -hi], 2), np.concatenate([hi, hr], 2)], 1)
    def cast(t):
        b = np.ascontiguousarray(t.astype(np.float32).astype(jnp.bfloat16)).view(np.uint16).astype(np.uint32)
        return b[..., 0::2, :] | (b[..., 1::2, :] << 16)
    pm = np.zeros((128, 128))
    for k1_ in range(R):
        for j in range(8):
            pm[k1_ * 8 + j, k1_ + R * j] = 1.0
    return cast(f1), cast(np.ascontiguousarray(fi.T)), cast(g), cast(gin), cast(pm)


def _cmul_w16(z, e, sgn):
    re, im = z
    e %= 16
    if e == 0:
        return z
    if e == 4:
        return (-sgn * im, sgn * re) if sgn == 1 else (im, -re)
    if e == 8:
        return (-re, -im)
    if e == 12:
        return (sgn * im, -sgn * re) if sgn == 1 else (-im, re)
    c = float(np.cos(2 * np.pi * e / 16))
    s = float(sgn * np.sin(2 * np.pi * e / 16))
    if e % 4 == 2:
        if (c > 0) == (s > 0):
            return ((re - im) * c, (re + im) * c)
        return ((re + im) * c, (im - re) * c)
    return (re * c - im * s, re * s + im * c)


def _dft4(a, b, c, d, sgn):
    s0 = (a[0] + c[0], a[1] + c[1])
    d0 = (a[0] - c[0], a[1] - c[1])
    s1 = (b[0] + d[0], b[1] + d[1])
    d1 = (b[0] - d[0], b[1] - d[1])
    y0 = (s0[0] + s1[0], s0[1] + s1[1])
    y2 = (s0[0] - s1[0], s0[1] - s1[1])
    if sgn > 0:
        y1 = (d0[0] - d1[1], d0[1] + d1[0])
        y3 = (d0[0] + d1[1], d0[1] - d1[0])
    else:
        y1 = (d0[0] + d1[1], d0[1] - d1[0])
        y3 = (d0[0] - d1[1], d0[1] + d1[0])
    return y0, y1, y2, y3


def _dft16(x, sgn):
    t = [None] * 4
    for b in range(4):
        t[b] = _dft4(x[b], x[4 + b], x[8 + b], x[12 + b], sgn)
    out = [None] * 16
    for c in range(4):
        u = [_cmul_w16(t[b][c], b * c, sgn) for b in range(4)]
        y = _dft4(u[0], u[1], u[2], u[3], sgn)
        for d in range(4):
            out[c + 4 * d] = y[d]
    return out


NEG = -1e9 * LOG2E
QSCALE = float(D ** -0.5) * LOG2E
HB = BQ // 2
KH = DC // 2
NB = S // BQ
U32 = jnp.uint32
OPLACE = {7: (0, 1, 2, 3, 4, 5, 6)}
CARRY = (7,)
GR = 16
ACOL = 384
UCH = 16


def _ds(start, size, mult=None):
    if not isinstance(start, int):
        start = pl.multiple_of(start, mult or size)
    return pl.ds(start, size)


def _ld(ref, pre, r0, nr, cols=slice(None)):
    return pltpu.bitcast(ref[pre + (_ds(r0 // 2, nr // 2, 8), cols)], BF16)


def _st(ref, pre, r0, val, cols=slice(None)):
    ref[pre + (_ds(r0 // 2, val.shape[0] // 2, 8), cols)] = pltpu.bitcast(val.astype(BF16), U32)


def _kernel(ax_hbm, wr_hbm, wi_hbm, x_hbm, c_hbm, wq_hbm, wuk_hbm, wuv_hbm, wo_hbm,
            f1_hbm, fi_hbm, g_hbm, gn_hbm, pm_hbm, out_hbm,
            ax_v, wr_v, wi_v, x_v, c_v, wq_v, wuk_v, wuv_v, wo_v,
            f1_v, fi_v, g_v, gn_v, pm_v, xt_v, wp_v,
            y_v, z_v, t_v, yf_v,
            q_v, k_v, v_v, ctx_v, wqb_v, bc_v, ac_v, xc_v, pa_v, pb_v,
            acc_v, ot_v, out_v,
            sem_a, sem_w, sem_wo, sem_o, sem_x):
    wq32 = wq_hbm.bitcast(U32)
    wuk32 = wuk_hbm.bitcast(U32)
    wuv32 = wuv_hbm.bitcast(U32)
    wo32 = wo_hbm.bitcast(U32)

    def wcopies(p):
        return (pltpu.make_async_copy(wq32.at[:, p, :], wq_v.at[p], sem_w.at[p, 0]),
                pltpu.make_async_copy(wuk32.at[:, p, :], wuk_v.at[p], sem_w.at[p, 1]),
                pltpu.make_async_copy(wuv32.at[:, p, :], wuv_v.at[p], sem_w.at[p, 2]))

    def wocopy(h):
        return pltpu.make_async_copy(wo32.at[h], wo_v.at[h], sem_wo.at[h])

    def ocopy(i):
        rows = _ds(i * BQ, BQ)
        cols = pl.ds(ACOL, 2 * M - ACOL)
        return pltpu.make_async_copy(out_v.at[rows, cols], out_hbm.at[rows, cols], sem_o.at[i])

    acopy = pltpu.make_async_copy(out_v.at[:, pl.ds(0, ACOL)], out_hbm.at[:, pl.ds(0, ACOL)], sem_a.at[0])

    def cp_ax(i):
        n = _ds(i * 512, 512)
        return pltpu.make_async_copy(ax_hbm.bitcast(U32).at[:, n], ax_v.at[:, n], sem_x.at[i])

    cp_f1 = pltpu.make_async_copy(f1_hbm, f1_v, sem_a.at[1])
    cp_g = pltpu.make_async_copy(g_hbm, g_v, sem_a.at[2])
    cp_gn = pltpu.make_async_copy(gn_hbm, gn_v, sem_a.at[3])
    cp_fi = pltpu.make_async_copy(fi_hbm, fi_v, sem_a.at[4])
    cp_x = pltpu.make_async_copy(x_hbm.bitcast(U32), xt_v, sem_a.at[5])
    cp_c = pltpu.make_async_copy(c_hbm.bitcast(U32), c_v, sem_a.at[6])
    cp_wr = pltpu.make_async_copy(wr_hbm, wr_v, sem_a.at[7])
    cp_wi = pltpu.make_async_copy(wi_hbm, wi_v, sem_a.at[8])
    cp_pm = pltpu.make_async_copy(pm_hbm, pm_v, sem_a.at[9])

    def _halves(w):
        return (pltpu.bitcast(w << 16, F32), pltpu.bitcast(w & U32(0xFFFF0000), F32))

    def combos(src, dst, i, width):
        ch = 16
        for r in range(0, HB // 2, ch):
            top = _ds(i * (BQ // 2) + r, ch, 8)
            bot = _ds(i * (BQ // 2) + HB // 2 + r, ch, 8)
            a11 = _halves(src[top, pl.ds(0, width)])
            a12 = _halves(src[top, pl.ds(width, width)])
            a21 = _halves(src[bot, pl.ds(0, width)])
            a22 = _halves(src[bot, pl.ds(width, width)])
            terms = ((a11, a22, 1), (a21, a22, 1), (a11, a12, 1), (a21, a11, -1), (a12, a22, -1))
            for j, (u, v, sg) in enumerate(terms):
                t = [u[e] + v[e] if sg > 0 else u[e] - v[e] for e in range(2)]
                dst[j, _ds(i * (HB // 2) + r, ch, 8), :] = pltpu.bitcast(
                    pltpu.pack_elementwise(t, packed_dtype=BF16), U32)

    def latent_combos(i):
        combos(c_v, ac_v, i, KH)

    def unpack_weights(p, odd):
        sh = (odd * 16).astype(U32) if not isinstance(odd, int) else U32(odd * 16)
        unf = lambda t: pltpu.bitcast(lax.shift_left(lax.shift_right_logical(t, sh), U32(16)), F32)
        for r in range(0, D, UCH):
            b1 = unf(wq_v[p, pl.ds(r, UCH), :])
            b11, b12 = b1[:, :128], b1[:, 128:]
            if D + r < M:
                b2 = unf(wq_v[p, pl.ds(D + r, UCH), :])
                b21, b22 = b2[:, :128], b2[:, 128:]
                cmb = (b11 + b22, b11, b12 - b22, b21 - b11, b22, b11 + b12, b21 + b22)
            else:
                zero = jnp.zeros_like(b11)
                cmb = (b11, b11, b12, -b11, zero, b11 + b12, zero)
            for j, t in enumerate(cmb):
                _st(wqb_v, (j,), r, t)
        for r in range(0, KH, UCH):
            b11 = unf(wuk_v[p, pl.ds(r, UCH), :])
            b21 = unf(wuk_v[p, pl.ds(KH + r, UCH), :])
            b12 = unf(wuv_v[p, pl.ds(r, UCH), :])
            b22 = unf(wuv_v[p, pl.ds(KH + r, UCH), :])
            for j, t in enumerate((b11 + b22, b11, b12 - b22, b21 - b11, b22, b11 + b12, b21 + b22)):
                _st(bc_v, (j,), r, t)

    def x_combos(i):
        combos(x_v, xc_v, i, D)

    def proj_q(i):
        top, bot, ar = i * BQ, i * BQ + HB, i * HB
        mm = lambda a, j: jnp.dot(a, _ld(wqb_v, (j,), 0, D), preferred_element_type=F32)
        xc = lambda j: _ld(xc_v, (j,), ar, HB)
        m7 = mm(xc(4), 6)
        m1 = mm(xc(0), 0)
        m4 = mm(_ld(x_v, (), bot, HB, pl.ds(D, D)), 3)
        m5 = mm(xc(2), 4)
        m3 = mm(_ld(x_v, (), top, HB, pl.ds(0, D)), 2)
        _st(q_v, (), top, jnp.concatenate([m1 + m4 - m5 + m7, m3 + m5], axis=1) * QSCALE)
        m2 = mm(xc(1), 1)
        m6 = mm(xc(3), 5)
        _st(q_v, (), bot, jnp.concatenate([m2 + m4, m1 - m2 + m3 + m6], axis=1) * QSCALE)

    def proj_kv(i):
        top, bot, ar = i * BQ, i * BQ + HB, i * HB
        mm = lambda a, j: jnp.dot(a, _ld(bc_v, (j,), 0, KH), preferred_element_type=F32)
        ac = lambda j: _ld(ac_v, (j,), ar, HB)
        m7 = mm(ac(4), 6)
        m1 = mm(ac(0), 0)
        m4 = mm(_ld(c_v, (), bot, HB, pl.ds(KH, KH)), 3)
        m5 = mm(ac(2), 4)
        _st(k_v, (), top, m1 + m4 - m5 + m7)
        m3 = mm(_ld(c_v, (), top, HB, pl.ds(0, KH)), 2)
        _st(v_v, (), top, m3 + m5)
        m2 = mm(ac(1), 1)
        _st(k_v, (), bot, m2 + m4)
        m6 = mm(ac(3), 5)
        _st(v_v, (), bot, m1 - m2 + m3 + m6)

    cp_ax(0).start()
    cp_f1.start()
    cp_ax(1).start()
    cp_f1.wait()

    def a1(i, carry):
        n = _ds(i * 512, 512)
        for step, cps in ((0, (cp_ax(2), cp_ax(3), cp_pm, cp_wr, cp_wi)), (2, (cp_g,)), (3, (cp_gn, cp_x))):
            @pl.when(i == step)
            def _():
                for cp in cps:
                    cp.start()
        cp_ax(i).wait()
        acc_v[:, n] = jnp.zeros((M, 512), F32)
        ctx_v[_ds(i * 256, 256), :] = jnp.zeros((256, D), U32)
        y_v[n, :] = lax.dot_general(_ld(ax_v, (), 0, M, n), _ld(f1_v, (), 0, M), TN, preferred_element_type=F32)
        return carry
    lax.fori_loop(0, 4, a1, 0)

    def radix(src, dst_store, sgn, filler):
        def body(i, carry):
            r0 = pl.multiple_of(i * 8, 8)
            for j in range(2):
                xs = [src(n1, r0, j) for n1 in range(R)]
                ys = _dft16(xs, sgn)
                for k1 in range(R):
                    dst_store(k1, r0, j, ys[k1])
            filler(i)
            return carry
        def body_u(i, carry):
            for d in range(2):
                body(i * 2 + d, carry)
            return carry
        lax.fori_loop(0, N2 // 8 // 2, body_u, 0)

    def src_f(n1, r0, j):
        rows = _ds(n1 * N2 + r0, 8)
        return (y_v[rows, pl.ds(j * 128, 128)], y_v[rows, pl.ds(DFP + j * 128, 128)])

    def dst_f(k1, r0, j, y):
        _st(z_v, (k1,), 2 * r0, jnp.concatenate(y, axis=0), pl.ds(j * 128, 128))

    def wperm(c):
        for part, wsrc in enumerate((wr_v, wi_v)):
            wt = wsrc[:, _ds(c * 128, 128)]
            r = lax.dot_general(_ld(pm_v, (), 0, 128), wt, NT, preferred_element_type=F32)
            r = jnp.pad(r, ((0, 0), (0, DFP - DF)))
            for k1 in range(R):
                wp_v[k1, _ds(part * N2 + c * 8, 8), :] = r[k1 * 8:(k1 + 1) * 8]

    for cp in (cp_pm, cp_wr, cp_wi):
        cp.wait()
    w0 = wcopies(0)
    cp_c.start()

    radix(src_f, dst_f, -1, wperm)

    def fwd(k1):
        return jnp.dot(_ld(g_v, (k1,), 0, 2 * N2), _ld(z_v, (k1,), 0, 2 * N2), preferred_element_type=F32)

    cp_g.wait()
    cp_gn.wait()
    cp_x.wait()
    for cp in (cp_fi, w0[0], w0[1], w0[2], wocopy(0), wocopy(1)):
        cp.start()

    def spec(m, carry):
        n = _ds(m * 256, 256)
        xt = jnp.concatenate([_ld(xt_v, (), 0, M, n), jnp.zeros((4 * 128 - M, 256), BF16)], axis=0)
        _st(x_v, (), m * 256, xt.T)
        xa = fwd(2 * m)
        xb = fwd(2 * m + 1)
        for k1, x2 in ((2 * m, xa), (2 * m + 1, xb)):
            wrf = wp_v[k1, 0:N2, :]
            wif = wp_v[k1, N2:2 * N2, :]
            xr, xi = x2[:N2], x2[N2:]
            ur = (xr * wrf - xi * wif).astype(BF16)
            ui = (xr * wif + xi * wrf).astype(BF16)
            u = jnp.concatenate([ur, ui], axis=0)
            t_v[k1] = jnp.dot(_ld(gn_v, (k1,), 0, 2 * N2), u, preferred_element_type=F32)
        return carry
    lax.fori_loop(0, R // 2, spec, 0)

    def src_i(k1, r0, j):
        return (t_v[k1, pl.ds(r0, 8), pl.ds(j * 128, 128)],
                t_v[k1, _ds(N2 + r0, 8), pl.ds(j * 128, 128)])

    def dst_i(n1, r0, j, y):
        rows = _ds(n1 * N2 + r0, 8)
        yf_v[rows, pl.ds(j * 128, 128)] = y[0]
        yf_v[rows, pl.ds(DFP + j * 128, 128)] = y[1]

    radix(src_i, dst_i, 1, lambda i: None)
    cp_fi.wait()
    cp_c.wait()

    def a5(i, carry):
        n = _ds(i * 512, 512)
        yt = lax.dot_general(_ld(fi_v, (), 0, M), yf_v[n, :].astype(BF16), NT,
                             preferred_element_type=F32).astype(BF16)
        out_v[n, pl.ds(0, ACOL)] = yt[:ACOL].T
        _st(ot_v, (), ACOL, yt[ACOL:], n)
        latent_combos(2 * i)
        latent_combos(2 * i + 1)
        x_combos(2 * i)
        x_combos(2 * i + 1)
        return carry
    lax.fori_loop(0, 4, a5, 0)
    acopy.start()
    for cp in w0:
        cp.wait()

    row = lax.broadcasted_iota(jnp.int32, (HB, HB), 0)
    col = lax.broadcasted_iota(jnp.int32, (HB, HB), 1)
    tri = col <= row
    p_bufs = (pa_v, pb_v)

    def oproj(i, wo):
        cols = pl.ds(i * BQ, BQ)
        acc_v[:, cols] += lax.dot_general(wo, _ld(ctx_v, (), i * BQ, BQ), NT, preferred_element_type=F32)

    def head(h, carry):
        p = h // 2
        odd = h % 2

        @pl.when(jnp.logical_and(odd == 0, p + 1 < H // 2))
        def _():
            for cp in wcopies(p + 1):
                cp.start()
            wocopy(h + 2).start()
            wocopy(h + 3).start()

        @pl.when(jnp.logical_and(odd == 0, h > 0))
        def _():
            for cp in wcopies(p):
                cp.wait()

        wocopy(h).wait()
        wo_prev = _ld(wo_v, (jnp.maximum(h - 1, 0),), 0, M)
        wo = _ld(wo_v, (h,), 0, M)
        unpack_weights(p, odd)
        for j in CARRY:
            oproj(j, wo_prev)
        proj_q(0)
        proj_kv(0)
        for i in range(NB):
            r0 = i * BQ
            l1 = r0 + HB
            q = _ld(q_v, (), r0, BQ)
            s1 = lax.dot_general(q, _ld(k_v, (), 0, l1), NT, preferred_element_type=F32)
            s2 = lax.dot_general(q[HB:], _ld(k_v, (), l1, HB), NT, preferred_element_type=F32)
            if i + 1 < NB:
                proj_q(i + 1)
                proj_kv(i + 1)
            for j in OPLACE.get(i, ()):
                oproj(j, wo)
            sdl = jnp.where(tri, s1[:HB, r0:], NEG)
            s_lo = jnp.concatenate([s1[:HB, :r0], sdl], axis=1) if i > 0 else sdl
            s_hi = jnp.concatenate([s1[HB:], jnp.where(tri, s2, NEG)], axis=1)
            pb = p_bufs[i % 2]
            ls = []
            for half, s_h in enumerate((s_lo, s_hi)):
                w = s_h.shape[1]
                for g in range(HB // GR):
                    sg = s_h[g * GR:(g + 1) * GR]
                    pg = jnp.exp2(sg - jnp.max(sg, axis=1, keepdims=True))
                    _st(pb, (), half * HB + g * GR, pg, pl.ds(0, w))
                    ls.append(jnp.sum(pg, axis=1, keepdims=True))
            l = jnp.concatenate(ls, axis=0)
            o = jnp.dot(_ld(pb, (), 0, BQ, pl.ds(0, l1)), _ld(v_v, (), 0, l1), preferred_element_type=F32)
            o2 = jnp.dot(_ld(pb, (), HB, HB, pl.ds(l1, HB)), _ld(v_v, (), l1, HB), preferred_element_type=F32)
            o = jnp.concatenate([o[:HB], o[HB:] + o2], axis=0)
            _st(ctx_v, (), r0, o * pl.reciprocal(l))
        return carry

    lax.fori_loop(0, H, head, 0)

    for j in CARRY:
        oproj(j, _ld(wo_v, (H - 1,), 0, M))
    for i in range(NB):
        cols = pl.ds(i * BQ, BQ)
        blk = jnp.concatenate([_ld(ot_v, (), ACOL, M - ACOL, cols), acc_v[:, cols].astype(BF16)], axis=0)
        out_v[cols, pl.ds(ACOL, 2 * M - ACOL)] = blk.T
        ocopy(i).start()
    acopy.wait()
    for i in range(NB):
        ocopy(i).wait()


@jax.jit
def pallas_concat_heads__spectral_gfnet__compressed_kv_cla__prompt_kernel(
        A_x, A_w_r, A_w_i, B_x, B_c_kv, B_w_q, B_w_uk, B_w_uv, B_w_o):
    f1, fi, g, gin, pm = _consts()
    packed = lambda *shape: pltpu.VMEM(shape[:-2] + (shape[-2] // 2, shape[-1]), U32)
    hbm = pl.BlockSpec(memory_space=pltpu.HBM)
    scratch = [
        packed(M, S),
        pltpu.VMEM((DF, S), BF16),
        pltpu.VMEM((DF, S), BF16),
        packed(S, 4 * 128),
        packed(S, DC),
        pltpu.VMEM((H // 2, M, D), U32),
        pltpu.VMEM((H // 2, DC, D), U32),
        pltpu.VMEM((H // 2, DC, D), U32),
        packed(H, M, D),
        packed(M, 2 * DFP),
        packed(M, 2 * DFP),
        packed(R, 2 * N2, 2 * N2),
        packed(R, 2 * N2, 2 * N2),
        packed(128, 128),
        packed(M, S),
        pltpu.VMEM((R, 2 * N2, DFP), F32),
        pltpu.VMEM((S, 2 * DFP), F32),
        packed(R, 2 * N2, DFP),
        pltpu.VMEM((R, 2 * N2, DFP), F32),
        pltpu.VMEM((S, 2 * DFP), F32),
        packed(S, D),
        packed(S, D),
        packed(S, D),
        packed(S, D),
        packed(7, D, D // 2),
        packed(7, KH, D),
        packed(5, S // 2, KH),
        packed(5, S // 2, D),
        packed(BQ, S),
        packed(BQ, S),
        pltpu.VMEM((M, S), F32),
        packed(2 * M, S),
        pltpu.VMEM((S, 2 * M), BF16),
        pltpu.SemaphoreType.DMA((10,)),
        pltpu.SemaphoreType.DMA((H // 2, 3)),
        pltpu.SemaphoreType.DMA((H,)),
        pltpu.SemaphoreType.DMA((NB,)),
        pltpu.SemaphoreType.DMA((4,)),
    ]
    out = pl.pallas_call(
        _kernel,
        out_shape=jax.ShapeDtypeStruct((S, 2 * M), BF16),
        in_specs=[hbm] * 14,
        out_specs=hbm,
        scratch_shapes=scratch,
        compiler_params=pltpu.CompilerParams(vmem_limit_bytes=120 * 2**20),
        name="fused",
    )(A_x.reshape(S, M).T, A_w_r.T, A_w_i.T,
      B_x.reshape(S, M).T, B_c_kv.reshape(S, DC), B_w_q, B_w_uk, B_w_uv, jnp.swapaxes(B_w_o, 1, 2),
      jnp.asarray(f1), jnp.asarray(fi), jnp.asarray(g), jnp.asarray(gin), jnp.asarray(pm))
    return out.reshape(1, S, 2 * M)
```
